```python
import os as _os
_os.environ.setdefault("JAX_PLATFORMS", "cpu")
import jax
import jax.numpy as jnp

def _softmax(x, axis=-1):
    return jax.nn.softmax(x, axis=axis)
def _gelu(x):
    return jax.nn.gelu(x, approximate=True)
def _silu(x):
    return jax.nn.silu(x)
def _sigmoid(x):
    return jax.nn.sigmoid(x)
def _layernorm(x, axis=-1, eps=1e-5):
    m = jnp.mean(x, axis=axis, keepdims=True)
    v = jnp.var(x, axis=axis, keepdims=True)
    return (x - m) / jnp.sqrt(v + eps)
def _scatter_add(tgt, idx, src, axis=0):
    return tgt.at[idx].add(src)
def _segment_sum(src, seg, n):
    return jax.ops.segment_sum(src, seg, n)
class _Rng:
    def __init__(self, key):
        self._k = key
    def _next(self):
        self._k, sub = jax.random.split(self._k)
        return sub
    def normal(self, shape):
        return jax.random.normal(self._next(), shape, dtype=jnp.bfloat16)
    def randint(self, lo, hi, shape):
        return jax.random.randint(self._next(), shape, lo, hi, dtype=jnp.int32)
    def uniform(self, shape, lo=0.0, hi=1.0):
        return jax.random.uniform(self._next(), shape, jnp.bfloat16, lo, hi)
    def permutation(self, n):
        return jax.random.permutation(self._next(), n)


kernel_name = 'standalone__mha_softmax__near_ridge'

def setup_inputs():
    _rng = _Rng(jax.random.key(int.from_bytes(__import__("os").urandom(4), "little")))
    _w = (lambda a: (lambda t: t.astype(jnp.bfloat16) if jnp.issubdtype(t.dtype, jnp.floating) else t)(jnp.asarray(a)))
    B, H, Sq, Sk, D = 32, 32, 288, 512, 128
    return {
        "q": _w((lambda *s: _rng.normal(s) * 0.4)(B, H, Sq, D)),
        "k": _w((lambda *s: _rng.normal(s) * 0.4)(B, H, Sk, D)),
        "v": _w((lambda *s: _rng.normal(s) * 0.05)(B, H, Sk, D)),
    }

def reference(q, k, v):
    scale = q.shape[-1] ** -0.5
    scores = jnp.einsum("bhqd,bhkd->bhqk", q, k) * scale
    p = _softmax(scores, axis=-1)
    return jnp.einsum("bhqk,bhkd->bhqd", p, v)
```

```python
import functools
import jax
import jax.numpy as jnp
from jax import lax
import jax.experimental.pallas as pl
import jax.experimental.pallas.tpu as pltpu

LOG2E = 1.4426950408889634


def make(C=8, NI=6, NPH=4, BK=5, OSPLIT=2, compute=True, head=None):

    @jax.jit
    def fn(q, k, v):
        B, H, Sq, D = q.shape
        Sk = k.shape[2]
        BH = B * H
        N = BH // C
        PC = N // NPH
        NO = PC + BK
        cexp = (D ** -0.5) * LOG2E
        OR = Sq // OSPLIT

        def kernel(q_hbm, k_hbm, v_hbm, o_hbm, qb, kb, vb, ob, rsem, wsem):
            def reads(j):
                s = j % NI
                return (pltpu.make_async_copy(k_hbm.at[:, j], kb.at[s], rsem.at[s]),
                        pltpu.make_async_copy(q_hbm.at[:, j], qb.at[s], rsem.at[s]),
                        pltpu.make_async_copy(v_hbm.at[:, j], vb.at[s], rsem.at[s]))

            def writes(j):
                s = j % NO
                return tuple(
                    pltpu.make_async_copy(ob.at[s, :, pl.ds(t * OR, OR)],
                                          o_hbm.at[:, j, pl.ds(t * OR, OR)], wsem.at[0])
                    for t in range(OSPLIT))

            def loop(lo, hi, f):
                def body(j, carry):
                    f(j)
                    return carry
                lax.fori_loop(lo, hi, body, 0)

            def start_reads(j):
                for cp in reads(j): cp.start()
            def wait_reads(j):
                for cp in reads(j): cp.wait()
            def start_writes(j):
                for cp in writes(j): cp.start()
            def wait_writes(j):
                for cp in writes(j): cp.wait()

            for j in range(NI):
                start_reads(j)

            def step(j):
                jp = j % PC
                base = j - jp
                last_phase = base == N - PC

                @pl.when(jp < PC - BK)
                def _():
                    wait_reads(j)

                @pl.when(jp == PC - BK)
                def _():
                    for t in range(BK):
                        wait_reads(j + t)
                    loop(jnp.maximum(base - BK, 0), j, start_writes)

                if compute:
                    s = j % NI
                    so = j % NO
                    for g in range(C):
                        sc = lax.dot_general(qb[s, g], kb[s, g], (((1,), (1,)), ((), ())),
                                             preferred_element_type=jnp.float32)
                        m = jnp.max(sc, axis=-1, keepdims=True)
                        p = jnp.exp2((sc - m) * cexp)
                        l = jnp.sum(p, axis=-1, keepdims=True)
                        o = jnp.dot(p.astype(jnp.bfloat16), vb[s, g],
                                    preferred_element_type=jnp.float32)
                        ob[so, g] = (o * pl.reciprocal(l, approx=False)).astype(ob.dtype)

                @pl.when(jp + NI < PC)
                def _():
                    start_reads(j + NI)

                @pl.when(jnp.logical_and(last_phase, jp >= PC - BK))
                def _():
                    start_writes(j)

                @pl.when(jnp.logical_and(jp == PC - 1, jnp.logical_not(last_phase)))
                def _():
                    loop(jnp.maximum(base - BK, 0), base + PC - BK, wait_writes)
                    for t in range(NI):
                        start_reads(j + 1 + t)

            loop(0, N, step)
            loop(max(N - PC - BK, 0), N, wait_writes)

        out = pl.pallas_call(
            kernel,
            in_specs=[pl.BlockSpec(memory_space=pl.ANY)] * 3,
            out_specs=pl.BlockSpec(memory_space=pl.ANY),
            out_shape=jax.ShapeDtypeStruct((C, N, Sq, D), q.dtype),
            scratch_shapes=[pltpu.VMEM((NI, C, Sq, D), q.dtype),
                            pltpu.VMEM((NI, C, Sk, D), k.dtype),
                            pltpu.VMEM((NI, C, Sk, D), v.dtype),
                            pltpu.VMEM((NO, C, Sq, D), q.dtype),
                            pltpu.SemaphoreType.DMA((NI,)),
                            pltpu.SemaphoreType.DMA((1,))],
            compiler_params=pltpu.CompilerParams(vmem_limit_bytes=120 * 1024 * 1024),
        )(q.reshape(C, N, Sq, D), k.reshape(C, N, Sk, D), v.reshape(C, N, Sk, D))
        return out.reshape(B, H, Sq, D)
    return fn

pallas_standalone__mha_softmax__near_ridge_kernel = make(NPH=2, NI=9, BK=8)
```

```python
import jax
import jax.numpy as jnp
from jax import lax
import jax.experimental.pallas as pl
import jax.experimental.pallas.tpu as pltpu

LOG2E = 1.4426950408889634


def make(C=8, NI=5, BK=3, W0=56, TH=5, WG=9, WR=128, compute=True, nosemcheck=False):

    @jax.jit
    def fn(q, k, v):
        B, H, Sq, D = q.shape
        Sk = k.shape[2]
        BH = B * H
        N = BH // C
        cexp = (D ** -0.5) * LOG2E
        NP = BH * Sq // (WG * WR)
        PPC = C * Sq // WR
        assert C * Sq % WR == 0 and BH * Sq % (WG * WR) == 0

        def kernel(q_hbm, k_hbm, v_hbm, o_hbm, qb, kb, vb, ob, rsem, tsem, wsem):
            def kv_reads(j):
                s = j % NI
                return [pltpu.make_async_copy(k_hbm.at[j], kb.at[s], rsem.at[s]),
                        pltpu.make_async_copy(v_hbm.at[j], vb.at[s], rsem.at[s])]

            def reads(j):
                s = j % NI
                return kv_reads(j) + [pltpu.make_async_copy(q_hbm.at[j], qb.at[s], rsem.at[s])]

            sl = (N - 1) % NI

            def last_main():
                return kv_reads(N - 1) + [
                    pltpu.make_async_copy(q_hbm.at[N - 1, pl.ds(0, C - TH)],
                                          qb.at[sl, pl.ds(0, C - TH)], rsem.at[sl])]

            def last_tail():
                return [pltpu.make_async_copy(q_hbm.at[N - 1, pl.ds(C - TH, TH)],
                                              qb.at[sl, pl.ds(C - TH, TH)], tsem)]

            def start_write(i):
                pltpu.make_async_copy(ob.at[:, i], o_hbm.at[:, i], wsem).start()

            def loop(lo, hi, f):
                def body(j, carry):
                    f(j)
                    return carry
                lax.fori_loop(lo, hi, body, 0)

            def start(cs):
                for cp in cs:
                    cp.start()

            def wait(cs):
                for cp in cs:
                    cp.wait()

            for j in range(NI):
                start(reads(j))

            def step(j):
                @pl.when(j < N - BK)
                def _():
                    wait(reads(j))

                @pl.when(j == N - BK)
                def _():
                    for t in range(N - BK, N - 1):
                        wait(reads(t))
                    wait(last_main())
                    loop(0, W0, start_write)
                    wait(last_tail())

                if compute:
                    s = j % NI
                    for g in range(C):
                        sc = lax.dot_general(qb[s, g], kb[s, g], (((1,), (1,)), ((), ())),
                                             preferred_element_type=jnp.float32)
                        m = jnp.max(sc, axis=-1, keepdims=True)
                        p = jnp.exp2((sc - m) * cexp)
                        l = jnp.sum(p, axis=-1, keepdims=True)
                        o = jnp.dot(p.astype(jnp.bfloat16), vb[s, g],
                                    preferred_element_type=jnp.float32)
                        r = pl.reciprocal(l, approx=True)
                        r = r * (2.0 - l * r)
                        res = (o * r).astype(ob.dtype)
                        lo = g * Sq
                        while lo < (g + 1) * Sq:
                            hi = min((lo // WR + 1) * WR, (g + 1) * Sq)
                            piece = j * PPC + lo // WR
                            ob[piece // NP, piece % NP, pl.ds(lo % WR, hi - lo), :] = (
                                res[lo - g * Sq:hi - g * Sq])
                            lo = hi

                @pl.when(j + NI < N - 1)
                def _():
                    start(reads(j + NI))

                @pl.when(j + NI == N - 1)
                def _():
                    start(last_main())
                    start(last_tail())

            loop(0, N, step)
            loop(W0, NP, start_write)
            pltpu.make_async_copy(ob, o_hbm, wsem).wait()

        out = pl.pallas_call(
            kernel,
            in_specs=[pl.BlockSpec(memory_space=pl.ANY)] * 3,
            out_specs=pl.BlockSpec(memory_space=pl.ANY),
            out_shape=jax.ShapeDtypeStruct((WG, NP, WR, D), q.dtype),
            scratch_shapes=[pltpu.VMEM((NI, C, Sq, D), q.dtype),
                            pltpu.VMEM((NI, C, Sk, D), k.dtype),
                            pltpu.VMEM((NI, C, Sk, D), v.dtype),
                            pltpu.VMEM((WG, NP, WR, D), q.dtype),
                            pltpu.SemaphoreType.DMA((NI,)),
                            pltpu.SemaphoreType.DMA(()),
                            pltpu.SemaphoreType.DMA(())],
            compiler_params=pltpu.CompilerParams(vmem_limit_bytes=112 * 1024 * 1024,
                                                 disable_semaphore_checks=nosemcheck),
        )(q.reshape(N, C, Sq, D), k.reshape(N, C, Sk, D), v.reshape(N, C, Sk, D))
        return out.reshape(B, H, Sq, D)
    return fn

pallas_standalone__mha_softmax__near_ridge_kernel = make()
```

```python
import jax
import jax.numpy as jnp
from jax import lax
import jax.experimental.pallas as pl
import jax.experimental.pallas.tpu as pltpu

_LOG2E = 1.4426950408889634


def _attention(q, k, v, *, heads, slots, backlog, tail_heads, groups, write_rows,
               early_writes, seg, interpret=False):
    B, H, Sq, D = q.shape
    Sk = k.shape[2]
    C, NI, BK, TH, WG, WR = heads, slots, backlog, tail_heads, groups, write_rows
    N = B * H // C
    WS = B * H * Sq // WG
    NW = WS // WR
    assert B * H == N * C and B * H * Sq == WG * WS
    assert WS % seg == 0 and (C * Sq) % seg == 0 and seg % 16 == 0 and Sq % 16 == 0
    assert WR % 16 == 0 and WS % 16 == 0 and 0 < TH < C and 1 < BK < NI <= N - 2
    assert (WG - 1) * WS + early_writes * WR <= (N - BK) * C * Sq
    exp2_scale = (D ** -0.5) * _LOG2E

    def loop(lo, hi, f):
        def body(i, carry):
            f(i)
            return carry
        lax.fori_loop(lo, hi, body, 0)

    def start(copies):
        for c in copies:
            c.start()

    def wait(copies):
        for c in copies:
            c.wait()

    def kernel(q_hbm, k_hbm, v_hbm, o_hbm, q_buf, k_buf, v_buf, o_buf, write_sem):
        def start_write(i):
            rows = pl.ds(pl.multiple_of(i * WR, 16), WR)
            pltpu.make_async_copy(o_buf.at[:, rows], o_hbm.at[:, rows], write_sem).start()

        def compute_chunk(j):
            s = j % NI
            for g in range(C):
                scores = lax.dot_general(q_buf[s, g], k_buf[s, g], (((1,), (1,)), ((), ())),
                                         preferred_element_type=jnp.float32)
                row_max = jnp.max(scores, axis=-1, keepdims=True)
                p = jnp.exp2((scores - row_max) * exp2_scale)
                denom = jnp.sum(p, axis=-1, keepdims=True)
                acc = jnp.dot(p.astype(v_buf.dtype), v_buf[s, g],
                              preferred_element_type=jnp.float32)
                out = (acc * pl.reciprocal(denom, full_range=False)).astype(o_buf.dtype)
                lo = g * Sq
                while lo < (g + 1) * Sq:
                    hi = min((lo // seg + 1) * seg, (g + 1) * Sq)
                    idx = j * (C * Sq // seg) + lo // seg
                    row = (idx % (WS // seg)) * seg + lo % seg
                    o_buf[idx // (WS // seg), pl.ds(pl.multiple_of(row, 16), hi - lo), :] = (
                        out[lo - g * Sq:hi - g * Sq])
                    lo = hi

        def read_and_compute(read_sems, tail_sem):
            def kv_reads(j):
                s = j % NI
                return [pltpu.make_async_copy(k_hbm.at[j], k_buf.at[s], read_sems.at[s]),
                        pltpu.make_async_copy(v_hbm.at[j], v_buf.at[s], read_sems.at[s])]

            def reads(j):
                s = j % NI
                return kv_reads(j) + [
                    pltpu.make_async_copy(q_hbm.at[j], q_buf.at[s], read_sems.at[s])]

            def last_q(lo, n, sem):
                return [pltpu.make_async_copy(q_hbm.at[N - 1, pl.ds(lo, n)],
                                              q_buf.at[(N - 1) % NI, pl.ds(lo, n)], sem)]

            def last_reads():
                return kv_reads(N - 1) + last_q(0, C - TH, read_sems.at[(N - 1) % NI])

            def last_tail():
                return last_q(C - TH, TH, tail_sem)

            for j in range(NI):
                start(reads(j))

            def step(j):
                @pl.when(j < N - BK)
                def _():
                    wait(reads(j))

                @pl.when(j == N - BK)
                def _():
                    for t in range(N - BK, N - 1):
                        wait(reads(t))
                    wait(last_reads())
                    loop(0, early_writes, start_write)
                    wait(last_tail())

                compute_chunk(j)

                @pl.when(j + NI < N - 1)
                def _():
                    start(reads(j + NI))

                @pl.when(j + NI == N - 1)
                def _():
                    start(last_reads())
                    start(last_tail())

            loop(0, N, step)

        pl.run_scoped(read_and_compute, pltpu.SemaphoreType.DMA((NI,)),
                      pltpu.SemaphoreType.DMA(()))
        loop(early_writes, NW, start_write)
        if WS % WR:
            rows = pl.ds(NW * WR, WS % WR)
            pltpu.make_async_copy(o_buf.at[:, rows], o_hbm.at[:, rows], write_sem).start()
        pltpu.make_async_copy(o_buf, o_hbm, write_sem).wait()

    out = pl.pallas_call(
        kernel,
        in_specs=[pl.BlockSpec(memory_space=pl.ANY)] * 3,
        out_specs=pl.BlockSpec(memory_space=pl.ANY),
        out_shape=jax.ShapeDtypeStruct((WG, WS, D), q.dtype),
        scratch_shapes=[pltpu.VMEM((NI, C, Sq, D), q.dtype),
                        pltpu.VMEM((NI, C, Sk, D), k.dtype),
                        pltpu.VMEM((NI, C, Sk, D), v.dtype),
                        pltpu.VMEM((WG, WS, D), q.dtype),
                        pltpu.SemaphoreType.DMA(())],
        compiler_params=pltpu.CompilerParams(vmem_limit_bytes=112 * 1024 * 1024),
        interpret=interpret,
    )(q.reshape(N, C, Sq, D), k.reshape(N, C, Sk, D), v.reshape(N, C, Sk, D))
    return out.reshape(B, H, Sq, D)


@jax.jit
def pallas_standalone__mha_softmax__near_ridge_kernel(
    q: jax.Array,
    k: jax.Array,
    v: jax.Array,
):
    return _attention(q, k, v, heads=8, slots=6, backlog=4, tail_heads=5, groups=9,
                      write_rows=112, early_writes=64, seg=128)
```
